```python
import os as _os
_os.environ.setdefault("JAX_PLATFORMS", "cpu")
import jax
import jax.numpy as jnp

def _softmax(x, axis=-1):
    return jax.nn.softmax(x, axis=axis)
def _gelu(x):
    return jax.nn.gelu(x, approximate=True)
def _silu(x):
    return jax.nn.silu(x)
def _sigmoid(x):
    return jax.nn.sigmoid(x)
def _layernorm(x, axis=-1, eps=1e-5):
    m = jnp.mean(x, axis=axis, keepdims=True)
    v = jnp.var(x, axis=axis, keepdims=True)
    return (x - m) / jnp.sqrt(v + eps)
def _scatter_add(tgt, idx, src, axis=0):
    return tgt.at[idx].add(src)
def _segment_sum(src, seg, n):
    return jax.ops.segment_sum(src, seg, n)
class _Rng:
    def __init__(self, key):
        self._k = key
    def _next(self):
        self._k, sub = jax.random.split(self._k)
        return sub
    def normal(self, shape):
        return jax.random.normal(self._next(), shape, dtype=jnp.bfloat16)
    def randint(self, lo, hi, shape):
        return jax.random.randint(self._next(), shape, lo, hi, dtype=jnp.int32)
    def uniform(self, shape, lo=0.0, hi=1.0):
        return jax.random.uniform(self._next(), shape, jnp.bfloat16, lo, hi)
    def permutation(self, n):
        return jax.random.permutation(self._next(), n)


kernel_name = 'standalone__gqa_softmax__decode'

def setup_inputs():
    _rng = _Rng(jax.random.key(int.from_bytes(__import__("os").urandom(4), "little")))
    _w = (lambda a: (lambda t: t.astype(jnp.bfloat16) if jnp.issubdtype(t.dtype, jnp.floating) else t)(jnp.asarray(a)))
    B, Hq, Hkv, Sq, Sk, D = 8, 32, 32, 1, 4096, 128
    return {
        "q": _w((lambda *s: _rng.normal(s) * 0.4)(B, Hq, Sq, D)),
        "k": _w((lambda *s: _rng.normal(s) * 0.4)(B, Hkv, Sk, D)),
        "v": _w((lambda *s: _rng.normal(s) * 0.05)(B, Hkv, Sk, D)),
    }

def reference(q, k, v):
    B, Hq, Sq, D = q.shape
    Hkv = k.shape[1]
    rep = Hq // Hkv
    k = jnp.repeat(k, rep, axis=1)
    v = jnp.repeat(v, rep, axis=1)
    scale = D ** -0.5
    scores = jnp.einsum("bhqd,bhkd->bhqk", q, k) * scale
    p = _softmax(scores, axis=-1)
    return jnp.einsum("bhqk,bhkd->bhqd", p, v)
```

```python
import functools

import jax
import jax.numpy as jnp
from jax import lax
import jax.experimental.pallas as pl
import jax.experimental.pallas.tpu as pltpu

_K_SLOTS = 3
_V_SLOTS = 2


def _decode_kernel(
    q_hbm, k_hbm, v_hbm, o_hbm,
    k_buf, v_buf, q_buf, q_f32, o_f32, o_buf,
    k_sem, v_sem, q_sem, o_sem,
    *, rows,
):
    n, _, d = k_hbm.shape
    scale = d ** -0.5

    def k_copy(i, slot):
        return pltpu.make_async_copy(k_hbm.at[i], k_buf.at[slot], k_sem.at[slot])

    def v_copy(i, slot):
        return pltpu.make_async_copy(v_hbm.at[i], v_buf.at[slot], v_sem.at[slot])

    q_copy = pltpu.make_async_copy(q_hbm, q_buf, q_sem)

    k_copy(0, 0).start()
    q_copy.start()
    for j in range(1, max(_K_SLOTS, _V_SLOTS + 1)):
        if j < min(_K_SLOTS, n):
            k_copy(j, j).start()
        if j - 1 < min(_V_SLOTS, n):
            v_copy(j - 1, j - 1).start()
    q_copy.wait()
    q_f32[...] = q_buf[...].astype(jnp.float32)

    def body(i, carry):
        ks = i % _K_SLOTS
        vs = i % _V_SLOTS
        q = q_f32[pl.ds(i * rows, rows), :].astype(q_buf.dtype)

        k_copy(i, ks).wait()
        s = lax.dot_general(
            q, k_buf[ks], (((1,), (1,)), ((), ())),
            preferred_element_type=jnp.float32,
        ) * scale

        @pl.when(i + _K_SLOTS < n)
        def _():
            k_copy(i + _K_SLOTS, ks).start()

        m = jnp.max(s, axis=-1, keepdims=True)
        p = jnp.exp(s - m)
        l = jnp.sum(p, axis=-1, keepdims=True)

        v_copy(i, vs).wait()
        o = jnp.dot(
            p.astype(v_buf.dtype), v_buf[vs], preferred_element_type=jnp.float32
        )

        @pl.when(i + _V_SLOTS < n)
        def _():
            v_copy(i + _V_SLOTS, vs).start()

        o_f32[pl.ds(i * rows, rows), :] = o / l
        return carry

    lax.fori_loop(0, n, body, 0)

    o_buf[...] = o_f32[...].astype(o_buf.dtype)
    o_copy = pltpu.make_async_copy(o_buf, o_hbm, o_sem)
    o_copy.start()
    o_copy.wait()


@jax.jit
def pallas_standalone__gqa_softmax__decode_kernel(
    q: jax.Array,
    k: jax.Array,
    v: jax.Array,
):
    B, Hq, Sq, D = q.shape
    _, Hkv, Sk, _ = k.shape
    n = B * Hkv
    rows = (Hq // Hkv) * Sq

    q2 = q.reshape(n * rows, D)
    k3 = k.reshape(n, Sk, D)
    v3 = v.reshape(n, Sk, D)

    out = pl.pallas_call(
        functools.partial(_decode_kernel, rows=rows),
        in_specs=[pl.BlockSpec(memory_space=pl.ANY)] * 3,
        out_specs=pl.BlockSpec(memory_space=pl.ANY),
        out_shape=jax.ShapeDtypeStruct(q2.shape, q.dtype),
        scratch_shapes=[
            pltpu.VMEM((_K_SLOTS, Sk, D), k.dtype),
            pltpu.VMEM((_V_SLOTS, Sk, D), v.dtype),
            pltpu.VMEM(q2.shape, q.dtype),
            pltpu.VMEM(q2.shape, jnp.float32),
            pltpu.VMEM(q2.shape, jnp.float32),
            pltpu.VMEM(q2.shape, q.dtype),
            pltpu.SemaphoreType.DMA((_K_SLOTS,)),
            pltpu.SemaphoreType.DMA((_V_SLOTS,)),
            pltpu.SemaphoreType.DMA(()),
            pltpu.SemaphoreType.DMA(()),
        ],
        compiler_params=pltpu.CompilerParams(vmem_limit_bytes=32 * 1024 * 1024),
    )(q2, k3, v3)
    return out.reshape(B, Hq, Sq, D)
```
